```python
import os as _os
_os.environ.setdefault("JAX_PLATFORMS", "cpu")
import jax
import jax.numpy as jnp

def _softmax(x, axis=-1):
    return jax.nn.softmax(x, axis=axis)
def _gelu(x):
    return jax.nn.gelu(x, approximate=True)
def _silu(x):
    return jax.nn.silu(x)
def _sigmoid(x):
    return jax.nn.sigmoid(x)
def _layernorm(x, axis=-1, eps=1e-5):
    m = jnp.mean(x, axis=axis, keepdims=True)
    v = jnp.var(x, axis=axis, keepdims=True)
    return (x - m) / jnp.sqrt(v + eps)
def _scatter_add(tgt, idx, src, axis=0):
    return tgt.at[idx].add(src)
def _segment_sum(src, seg, n):
    return jax.ops.segment_sum(src, seg, n)
class _Rng:
    def __init__(self, key):
        self._k = key
    def _next(self):
        self._k, sub = jax.random.split(self._k)
        return sub
    def normal(self, shape):
        return jax.random.normal(self._next(), shape, dtype=jnp.bfloat16)
    def randint(self, lo, hi, shape):
        return jax.random.randint(self._next(), shape, lo, hi, dtype=jnp.int32)
    def uniform(self, shape, lo=0.0, hi=1.0):
        return jax.random.uniform(self._next(), shape, jnp.bfloat16, lo, hi)
    def permutation(self, n):
        return jax.random.permutation(self._next(), n)


kernel_name = 'parallel_sum__sliding_block__moe_arch_mod__prompt'

def setup_inputs():
    _rng = _Rng(jax.random.key(int.from_bytes(__import__("os").urandom(4), "little")))
    _w = (lambda a: (lambda t: t.astype(jnp.bfloat16) if jnp.issubdtype(t.dtype, jnp.floating) else t)(jnp.asarray(a)))
    def _A_setup():
        B, S, D = 1, 2048, 512
        return {
            "x": _w((lambda *s: _rng.normal(s) * 0.05)(B, S, D)),
            "wqkv": _w((lambda *s: _rng.normal(s) * 0.05)(D, 3 * D)),
            "wo": _w((lambda *s: _rng.normal(s) * 0.05)(D, D)),
        }
    _A_in = _A_setup()

    def _B_setup():
        B, S, D, F, C = 1, 2048, 512, 1376, 1
        return {
            "x": _w((lambda *s: _rng.normal(s) * 0.05)(B, S, D)),
            "w_r": _w((lambda *s: _rng.normal(s) * 0.05)(D)),
            "w_gate": _w((lambda *s: _rng.normal(s) * 0.05)(D, F)),
            "w_up": _w((lambda *s: _rng.normal(s) * 0.05)(D, F)),
            "w_down": _w((lambda *s: _rng.normal(s) * 0.05)(F, D)),
        }
    _B_in = _B_setup()

    return {
        "A_x": _A_in["x"],
        "A_wqkv": _A_in["wqkv"],
        "A_wo": _A_in["wo"],
        "B_x": _B_in["x"],
        "B_w_r": _B_in["w_r"],
        "B_w_gate": _B_in["w_gate"],
        "B_w_up": _B_in["w_up"],
        "B_w_down": _B_in["w_down"],
    }

def reference(A_x, A_wqkv, A_wo, B_x, B_w_r, B_w_gate, B_w_up, B_w_down):
    def _A_ref(x, wqkv, wo):
        B, S, D = x.shape
        H = 32; Dh = D // H; W = 256
        qkv = (lambda x, *d: x.transpose(*d))((x @ wqkv).reshape(B, S, 3, H, Dh), 2, 0, 3, 1, 4)
        q, k, v = qkv[0], qkv[1], qkv[2]
        scores = jnp.einsum("bhqd,bhkd->bhqk", q, k) * (Dh ** -0.5)
        idx = jnp.arange(S)
        mask = (idx[:, None] - idx[None, :] >= 0) & (idx[:, None] - idx[None, :] < W)
        scores = jnp.where(mask[None, None], scores, -1e9)
        p = _softmax(scores, axis=-1)
        o = jnp.einsum("bhqk,bhkd->bhqd", p, v)
        return (lambda x, *d: x.transpose(*d))(o, 0, 2, 1, 3).reshape(B, S, D) @ wo

    def _B_ref(x, w_r, w_gate, w_up, w_down):
        B, S, D = x.shape
        C = 1
        r = x @ w_r
        idx = jnp.argsort(-r, axis=-1)[:, :C]
        idx_e = jnp.repeat(idx.reshape(B, C, 1), D, axis=2)
        x_sel = jnp.take_along_axis(x, idx_e, axis=1)
        g = _silu(x_sel @ w_gate)
        u = x_sel @ w_up
        y = (g * u) @ w_down
        r_sel = _sigmoid(jnp.take_along_axis(r, idx, axis=1))
        y = y * r_sel.reshape(B, C, 1)
        b_off = (jnp.arange(B) * S).reshape(B, 1)
        flat_idx = (idx + b_off).reshape(B * C)
        zero = (x * 0.0).reshape(B * S, D)
        upd = _scatter_add(zero, flat_idx, y.reshape(B * C, D), axis=0)
        return x + upd.reshape(B, S, D)

    x = A_x
    xn = _layernorm(x, axis=-1)
    return x + _A_ref(xn, A_wqkv, A_wo) + _B_ref(xn, B_w_r, B_w_gate, B_w_up, B_w_down)
```

```python
import functools
import numpy as np
import jax
import jax.numpy as jnp
from jax import lax
from jax.experimental import pallas as pl
from jax.experimental.pallas import tpu as pltpu

S = 2048
D = 512
H = 32
DH = 16
W = 256
F = 1376
QB = 128
NEG = -1e30
LOG2E = 1.4426950408889634
QSCALE = (DH ** -0.5) * LOG2E
f32 = jnp.float32
bf16 = jnp.bfloat16


def _rbf(x):
    return x.astype(bf16).astype(f32)


def _ln(x):
    xf = x.astype(f32)
    mean = jnp.mean(xf, axis=-1, keepdims=True)
    c = xf - mean
    var = jnp.mean(c * c, axis=-1, keepdims=True)
    m = _rbf(mean)
    v = _rbf(var)
    eps = float(np.float32(np.asarray(1e-5, dtype=jnp.bfloat16)))
    den = _rbf(jnp.sqrt(_rbf(v + eps)))
    xc = _rbf(xf - m)
    return (xc * (1.0 / den)).astype(bf16)


def _window(half, nkb):
    if nkb is None:
        w0 = 64 * half
    else:
        w0 = max(64 * half, 256 - 128 * nkb)
    return w0, 64 * half + 320


def _phase_a(q_ref, k_ref, qrow, krow0, g, half, nkb):
    w0, w1 = _window(half, nkb)
    nrows = w1 - w0
    qa = q_ref[pl.ds(qrow + 64 * half, 64), g * 128:(g + 1) * 128]
    qi = pltpu.bitcast(qa, jnp.uint32)
    hid = lax.broadcasted_iota(jnp.int32, (32, 128), 1) >> 4
    parts = []
    for hh in range(8):
        h = hh if half == 0 else (hh ^ 1)
        msk = jnp.where(hid == h, jnp.uint32(0xFFFFFFFF), jnp.uint32(0))
        parts.append(pltpu.bitcast(qi & msk, bf16))
    qbd = jnp.concatenate(parts, axis=0)
    kblk = k_ref[pl.ds(krow0 + w0, nrows), g * 128:(g + 1) * 128]
    st = lax.dot_general(kblk, qbd, (((1,), (1,)), ((), ())), preferred_element_type=f32)
    j = lax.broadcasted_iota(jnp.int32, (64, 512), 1) & 63
    r = lax.broadcasted_iota(jnp.int32, (64, 512), 0)
    pieces = []
    for c in range(nrows // 64):
        i0 = c * 64 + w0 - 64 * half
        sc = st[c * 64:(c + 1) * 64]
        if i0 == 0:
            sc = jnp.where(r > j, sc, NEG)
        elif i0 == 256:
            sc = jnp.where(r <= j, sc, NEG)
        pieces.append(sc)
    m = pieces[0]
    for p in pieces[1:]:
        m = jnp.maximum(m, p)
    m = jnp.max(m, axis=0, keepdims=True)
    return pieces, m


def _phase_b(pieces, m, vt_ref, vblk0, g, half, nkb):
    w0, w1 = _window(half, nkb)
    t0 = w0 // 128
    padlo = w0 - t0 * 128
    padhi = 384 - w1
    outs = []
    for p in range(4):
        sl = slice(p * 128, (p + 1) * 128)
        ps = [jnp.exp2(pc[:, sl] - m[:, sl]) for pc in pieces]
        l = ps[0]
        for x in ps[1:]:
            l = l + x
        l = jnp.sum(l, axis=0, keepdims=True)
        parts = []
        if padlo:
            parts.append(jnp.zeros((padlo, 128), bf16))
        parts += [x.astype(bf16) for x in ps]
        if padhi:
            parts.append(jnp.zeros((padhi, 128), bf16))
        pt = jnp.concatenate(parts, axis=0)
        hp = g * 8 + 2 * p
        vt = jnp.concatenate(
            [vt_ref[vblk0 + t, hp * DH:(hp + 2) * DH, :] for t in range(t0, 3)], axis=1)
        o = jnp.dot(vt, pt, preferred_element_type=f32) * (1.0 / l)
        outs.append(o)
    return outs


def _store_o(ot_ref, g, oas, obs):
    lo = lax.broadcasted_iota(jnp.int32, (DH, 128), 1) < 64
    for p in range(4):
        hp = g * 8 + 2 * p
        oa, ob = oas[p], obs[p]
        o0 = jnp.where(lo, oa[:DH], ob[:DH])
        o1 = pltpu.roll(jnp.where(lo, ob[DH:], oa[DH:]), 64, 1)
        ot_ref[hp * DH:(hp + 1) * DH, :] = o0.astype(bf16)
        ot_ref[(hp + 1) * DH:(hp + 2) * DH, :] = o1.astype(bf16)


def _attn_block(q_ref, k_ref, vt_ref, ot_ref, qrow, krow0, vblk0, nkb, swp):
    units = [(g, half) for g in range(4) for half in range(2)]
    res = {}
    if swp:
        a = _phase_a(q_ref, k_ref, qrow, krow0, *units[0], nkb)
        for n, (g, half) in enumerate(units):
            cur = a
            if n + 1 < len(units):
                a = _phase_a(q_ref, k_ref, qrow, krow0, *units[n + 1], nkb)
            res[(g, half)] = _phase_b(*cur, vt_ref, vblk0, g, half, nkb)
            if half == 1:
                _store_o(ot_ref, g, res.pop((g, 0)), res.pop((g, 1)))
    else:
        for (g, half) in units:
            cur = _phase_a(q_ref, k_ref, qrow, krow0, g, half, nkb)
            res[(g, half)] = _phase_b(*cur, vt_ref, vblk0, g, half, nkb)
            if half == 1:
                _store_o(ot_ref, g, res.pop((g, 0)), res.pop((g, 1)))


def _kernel(x_ref, wqkv_ref, wo_ref, wr_ref, wg_hbm, wu_hbm, wd_hbm,
            o_ref,
            q_ref, k_ref, vt_ref, ot_ref, xn_ref, wvt_ref, r_ref,
            wg_ref, wu_ref, wd_ref, sems, *, nq, swp):
    i = pl.program_id(0)
    nsteps = pl.num_programs(0)

    def ffn_copies():
        return (pltpu.make_async_copy(wg_hbm, wg_ref, sems.at[0]),
                pltpu.make_async_copy(wu_hbm, wu_ref, sems.at[1]),
                pltpu.make_async_copy(wd_hbm, wd_ref, sems.at[2]))

    @pl.when(i == 0)
    def _init():
        for c in ffn_copies():
            c.start()
        vt_ref[0] = jnp.zeros((D, 128), bf16)
        vt_ref[1] = jnp.zeros((D, 128), bf16)
        wvt_ref[0:D, :] = wqkv_ref[:, 2 * D:3 * D].T
        wvt_ref[D:D + 16, :] = jnp.broadcast_to(wr_ref[...], (16, D))

    for b in range(nq):
        blk = i * nq + b
        row = pl.multiple_of(blk * QB, QB)
        x = x_ref[b * QB:(b + 1) * QB, :]
        xn = _ln(x)
        xn_ref[pl.ds(row, QB), :] = xn
        qk = jnp.dot(xn, wqkv_ref[:, 0:2 * D], preferred_element_type=f32)
        q_ref[b * QB:(b + 1) * QB, :] = (qk[:, :D] * QSCALE).astype(bf16)
        k_ref[pl.ds(row + W, QB), :] = qk[:, D:].astype(bf16)
        vr = lax.dot_general(wvt_ref[...], xn, (((1,), (1,)), ((), ())),
                             preferred_element_type=f32)
        vt_ref[blk + 2] = vr[:D].astype(bf16)
        r_ref[blk] = vr[D:D + 8]

    for b in range(nq):
        blk = i * nq + b
        row = pl.multiple_of(blk * QB, QB)

        def full():
            _attn_block(q_ref, k_ref, vt_ref, ot_ref, b * QB, row, blk, None, swp)

        if nq == 1:
            @pl.when(i == 0)
            def _():
                _attn_block(q_ref, k_ref, vt_ref, ot_ref, 0, 0, 0, 0, swp)

            @pl.when(i == 1)
            def _():
                _attn_block(q_ref, k_ref, vt_ref, ot_ref, 0, QB, 1, 1, swp)

            pl.when(i >= 2)(full)
        else:
            if b < 2:
                @pl.when(i == 0)
                def _():
                    _attn_block(q_ref, k_ref, vt_ref, ot_ref, b * QB, b * QB, b, b, swp)

                pl.when(i > 0)(full)
            else:
                full()

        ao = lax.dot_general(ot_ref[...], wo_ref[...], (((0,), (0,)), ((), ())),
                             preferred_element_type=f32)
        x = x_ref[b * QB:(b + 1) * QB, :].astype(f32)
        xn = xn_ref[pl.ds(row, QB), :].astype(f32)
        o_ref[pl.ds(row, QB), :] = (x + ao + xn).astype(bf16)

    @pl.when(i == nsteps - 1)
    def _tail():
        for c in ffn_copies():
            c.wait()
        r = _rbf(r_ref[...])
        pos = (lax.broadcasted_iota(jnp.int32, r.shape, 0) * 128
               + lax.broadcasted_iota(jnp.int32, r.shape, 2))
        rmax = jnp.max(jnp.max(r, axis=0), axis=1, keepdims=True)
        cand = jnp.where(r == rmax[None], pos, S)
        idx = jnp.min(cand)
        g16 = pl.multiple_of((idx // 16) * 16, 16)
        xs = xn_ref[pl.ds(g16, 16), :]
        nt = (((1,), (1,)), ((), ()))
        g = lax.dot_general(xs, wg_ref[...], nt, preferred_element_type=f32)
        g = _rbf(g)
        g = _rbf(g * jax.nn.sigmoid(g))
        u = _rbf(lax.dot_general(xs, wu_ref[...], nt, preferred_element_type=f32))
        hmid = (g * u).astype(bf16)
        y = _rbf(jnp.dot(hmid, wd_ref[...], preferred_element_type=f32))
        gate = _rbf(jax.nn.sigmoid(rmax[0:1, :]))
        y = _rbf(y * gate)
        rows = lax.broadcasted_iota(jnp.int32, (16, D), 0)
        y = jnp.where(rows == (idx - g16), y, 0.0)
        cur = o_ref[pl.ds(g16, 16), :].astype(f32)
        o_ref[pl.ds(g16, 16), :] = (cur + y).astype(bf16)


def make(nq=1, swp=True, pin=True):
    kern = functools.partial(_kernel, nq=nq, swp=swp)

    @jax.jit
    def fn(A_x, A_wqkv, A_wo, B_x, B_w_r, B_w_gate, B_w_up, B_w_down):
        x = A_x.reshape(S, D)
        wr = B_w_r.reshape(1, D)
        nsteps = S // (QB * nq)
        args = [x, A_wqkv, A_wo, wr, B_w_gate.T, B_w_up.T, B_w_down]
        if pin:
            args = [pltpu.with_memory_space_constraint(a, pltpu.HBM) for a in args]
        out = pl.pallas_call(
            kern,
            grid=(nsteps,),
            in_specs=[
                pl.BlockSpec((QB * nq, D), lambda i: (i, 0)),
                pl.BlockSpec((D, 3 * D), lambda i: (0, 0)),
                pl.BlockSpec((D, D), lambda i: (0, 0)),
                pl.BlockSpec((1, D), lambda i: (0, 0)),
                pl.BlockSpec(memory_space=pl.ANY),
                pl.BlockSpec(memory_space=pl.ANY),
                pl.BlockSpec(memory_space=pl.ANY),
            ],
            out_specs=pl.BlockSpec((S, D), lambda i: (0, 0)),
            out_shape=jax.ShapeDtypeStruct((S, D), bf16),
            scratch_shapes=[
                pltpu.VMEM((QB * nq, D), bf16),
                pltpu.VMEM((S + W, D), bf16),
                pltpu.VMEM((S // 128 + 2, D, 128), bf16),
                pltpu.VMEM((D, 128), bf16),
                pltpu.VMEM((S, D), bf16),
                pltpu.VMEM((D + 16, D), bf16),
                pltpu.VMEM((S // 128, 8, 128), f32),
                pltpu.VMEM((F, D), bf16),
                pltpu.VMEM((F, D), bf16),
                pltpu.VMEM((F, D), bf16),
                pltpu.SemaphoreType.DMA((3,)),
            ],
            compiler_params=pltpu.CompilerParams(
                dimension_semantics=("arbitrary",),
                vmem_limit_bytes=64 * 1024 * 1024),
            name=f"k2_nq{nq}_swp{int(swp)}",
        )(*args)
        return out.reshape(1, S, D)

    return fn


_fn = make(4, True)


@jax.jit
def pallas_parallel_sum__sliding_block__moe_arch_mod__prompt_kernel(
    A_x: jax.Array,
    A_wqkv: jax.Array,
    A_wo: jax.Array,
    B_x: jax.Array,
    B_w_r: jax.Array,
    B_w_gate: jax.Array,
    B_w_up: jax.Array,
    B_w_down: jax.Array,
):
    return _fn(A_x, A_wqkv, A_wo, B_x, B_w_r, B_w_gate, B_w_up, B_w_down)
```

```python
import functools

import numpy as np
import jax
import jax.numpy as jnp
from jax import lax
from jax.experimental import pallas as pl
from jax.experimental.pallas import tpu as pltpu

S = 2048
D = 512
H = 32
DH = 16
W = 256
F = 1376
QB = 128
NB = S // QB
NEG = -1e30
QSCALE = (DH ** -0.5) * 1.4426950408889634
EPS_BF16 = float(np.float32(np.asarray(1e-5, dtype=jnp.bfloat16)))
f32 = jnp.float32
bf16 = jnp.bfloat16
u32 = jnp.uint32
NT = (((1,), (1,)), ((), ()))
TN = (((0,), (0,)), ((), ()))

UNITS = [(g, half) for g in range(4) for half in range(2)]

PROG_FIRST = ("g0 p0.1 p0.0 g1 a0.1 p1.0 a0.0 p1.1 a1.0 b0.0 a1.1 b1.0 b0.1 a2.0 a2.1 b1.1 a3.1 b2.0 "
              "g2 a3.0 p2.0 g3 p2.1 b2.1 p3.1 a4.0 a5.0 p3.0 b3.1 b3.0 a4.1 a5.1 b4.0 b5.0 a6.0 a7.0 b4.1 "
              "w b5.1 l b6.0 a6.1 a7.1 q0 q1 v0 b7.0 q2 v3 b6.1 n v1 q3 b7.1 O.0 O.1 v2").split()
PROG_LOOP = "a1 b0 a2 b1 a3 b2 a4 b3 a5 b4 a6 b5 a7 l q0 b6 q1 v3 v0 v2 b7 q2 v1 n O q3".split()
PROG_LAST = "tg tu a1 b0 a2 b1 a3 b2 a4 b3 a5 b4 a6 b5 a7 b6 b7 f O".split()
LOOP_SLOTS = 3
ALL_SLOTS = 4


def _rbf(x):
    return x.astype(bf16).astype(f32)


def _pk(x):
    return pltpu.bitcast(x, u32)


def _up(x):
    return pltpu.bitcast(x, bf16)


def _prow(start, n):
    if isinstance(start, int):
        return pl.ds(start // 2, n // 2)
    return pl.ds(pl.multiple_of(start // 2, 8), n // 2)


def _rows(blk):
    if isinstance(blk, int):
        return pl.ds(blk * QB, QB)
    return pl.ds(pl.multiple_of(blk * QB, QB), QB)


def _layernorm(x):
    xf = x.astype(f32)
    mean = jnp.mean(xf, axis=-1, keepdims=True)
    c = xf - mean
    var = jnp.mean(c * c, axis=-1, keepdims=True)
    den = _rbf(jnp.sqrt(_rbf(_rbf(var) + EPS_BF16)))
    xc = _rbf(xf - _rbf(mean))
    return (xc * (1.0 / den)).astype(bf16)


class _Ctx:
    pass


def _ln_block(R, blk):
    xn = _layernorm(R.x[_rows(blk), :])
    R.xn[_prow(blk * QB, QB), :] = _pk(xn)
    return xn


def _proj_k(R, blk, xn, g):
    c0, c1 = g * 128, (g + 1) * 128
    kk = jnp.dot(xn, _up(R.wk[:, c0:c1]), preferred_element_type=f32)
    R.k[_prow((blk + 2) * QB, QB), c0:c1] = _pk(kk.astype(bf16))


def _proj_qv(R, blk, xn, g):
    lhs = [_up(R.wqv[g * 64:(g + 1) * 64, :]), _up(R.wqv[D // 2 + g * 64:D // 2 + (g + 1) * 64, :])]
    if g == 3:
        lhs.append(_up(R.wqv[D:D + 8, :]))
    qv = lax.dot_general(jnp.concatenate(lhs, axis=0), xn, NT, preferred_element_type=f32)
    qt = _pk((qv[0:128] * QSCALE).astype(bf16))
    parts = [qt[8 * h:8 * h + 8] if h % 2 == 0 else pltpu.roll(qt[8 * h:8 * h + 8], 64, 1) for h in range(8)]
    R.q[blk, 64 * g:64 * (g + 1), :] = jnp.concatenate(parts, axis=0)
    R.vt[blk + 2, g * 64:(g + 1) * 64, :] = _pk(qv[128:256].astype(bf16))
    if g == 3:
        R.r[blk] = qv[256:264]


def _scores(R, blk, g, half, slot):
    w0 = 64 * half
    lo = lax.broadcasted_iota(jnp.int32, (8, 128), 1) < 64
    mlo = jnp.where(lo, u32(0xFFFFFFFF), u32(0))
    mhi = jnp.where(lo, u32(0), u32(0xFFFFFFFF))
    ma, mb = (mlo, mhi) if half == 0 else (mhi, mlo)
    qcols = []
    for p in range(4):
        h0 = 8 * g + 2 * p
        a = R.q[blk, 8 * h0:8 * h0 + 8, :] & ma
        b = R.q[blk, 8 * h0 + 8:8 * h0 + 16, :] & mb
        rows = []
        if p > 0:
            rows.append(jnp.zeros((16 * p, 128), u32))
        rows += [a, b]
        if p < 3:
            rows.append(jnp.zeros((48 - 16 * p, 128), u32))
        qcols.append(jnp.concatenate(rows, axis=0))
    qbd = _up(jnp.concatenate(qcols, axis=1))
    c_lo = max(0, (W - QB * blk - w0) // 64) if isinstance(blk, int) else 0
    kblk = _up(R.k[_prow(blk * QB + w0 + 64 * c_lo, 320 - 64 * c_lo), g * 128:(g + 1) * 128])
    st = jnp.dot(kblk, qbd, preferred_element_type=f32)
    cols, ms = [], []
    for p in range(4):
        pieces, pm = [], None
        for c in range(5):
            if c < c_lo:
                pieces.append(None)
                continue
            sc = st[(c - c_lo) * 64:(c - c_lo + 1) * 64, p * 128:(p + 1) * 128]
            if c == 0:
                sc = sc + R.bias[0:64, :]
            elif c == 4:
                sc = sc + R.bias[64:128, :]
            pieces.append(sc)
            cm = jnp.max(sc.reshape(8, 8, 128), axis=0)
            pm = cm if pm is None else jnp.maximum(pm, cm)
        cols.append(pieces)
        ms.append(jnp.max(pm, axis=0, keepdims=True))
    R.dep = [[None if cols[p][c] is None else cols[p][c][0:8, :] for c in range(5)] for p in range(4)]
    for p in range(4):
        for c in range(5):
            if cols[p][c] is not None:
                R.s[slot, c * 64:(c + 1) * 64, p * 128:(p + 1) * 128] = cols[p][c]
        R.m[slot, :, p * 128:(p + 1) * 128] = jnp.broadcast_to(ms[p], (8, 128))


def _softmax_pv(R, blk, g, half, slot, pace):
    dep, R.dep = R.dep, None
    w0 = 64 * half
    cols = [[R.s[slot, c * 64:(c + 1) * 64, p * 128:(p + 1) * 128] for c in range(5)] for p in range(4)]
    ms = [R.m[slot, 0:1, p * 128:(p + 1) * 128] for p in range(4)]
    accs, ls = [None] * 4, [None] * 4
    z = jnp.zeros((64, 128), f32)
    first_valid = W - QB * blk if isinstance(blk, int) else 0
    for t in range(3):
        for p in range(4):
            es = []
            for c2 in range(2):
                wrow = 128 * t + 64 * c2
                c = (wrow - w0) // 64
                if c < 0 or c > 4 or wrow < first_valid:
                    es.append(z)
                    continue
                cd = c - (pace or 0)
                if pace is not None and dep is not None and 0 <= cd < 5 and dep[p][cd] is not None:
                    mc = (ms[p] + 0.0 * dep[p][cd])[None]
                    e = jnp.exp2(cols[p][c].reshape(8, 8, 128) - mc).reshape(64, 128)
                else:
                    e = jnp.exp2(cols[p][c] - ms[p])
                es.append(e)
                part = jnp.sum(e.reshape(8, 8, 128), axis=0)
                ls[p] = part if ls[p] is None else ls[p] + part
            if 128 * (t + 1) <= first_valid:
                continue
            hp = g * 8 + 2 * p
            pt = jnp.concatenate(es, axis=0).astype(bf16)
            vt = _up(R.vt[blk + t, hp * (DH // 2):(hp + 2) * (DH // 2), :])
            o = jnp.dot(vt, pt, preferred_element_type=f32)
            accs[p] = o if accs[p] is None else accs[p] + o
    return [accs[p] * (1.0 / jnp.sum(ls[p], axis=0, keepdims=True)) for p in range(4)]


def _store_o(R, slot, g, oas, obs):
    lo = lax.broadcasted_iota(jnp.int32, (DH, 128), 1) < 64
    for p in range(4):
        hp = g * 8 + 2 * p
        oa, ob = oas[p], obs[p]
        o0 = jnp.where(lo, oa[:DH], ob[:DH])
        o1 = pltpu.roll(jnp.where(lo, ob[DH:], oa[DH:]), 64, 1)
        R.ot[slot, hp * (DH // 2):(hp + 2) * (DH // 2), :] = _pk(jnp.concatenate([o0, o1], axis=0).astype(bf16))


def _outproj(R, blk):
    ao = lax.dot_general(_up(R.ot[blk % 2]), _up(R.wo[...]), TN, preferred_element_type=f32)
    x = R.x[_rows(blk), :].astype(f32)
    xn = _up(R.xn[_prow(blk * QB, QB), :]).astype(f32)
    R.out[_rows(blk), :] = (x + ao + xn).astype(bf16)


def _transpose_ffn(src, dst):
    for j in range(pl.cdiv(F, 128)):
        n = min(128, F - 128 * j)
        dst[:, 128 * j:128 * j + n] = _pk(src[128 * j:128 * j + n, :].T)


def _route_ffn(R):
    r = _rbf(R.r[...])
    pos = (lax.broadcasted_iota(jnp.int32, r.shape, 0) * QB + lax.broadcasted_iota(jnp.int32, r.shape, 2))
    rmax = jnp.max(jnp.max(r, axis=0), axis=1, keepdims=True)
    idx = jnp.minimum(jnp.min(jnp.where(r == rmax[None], pos, S)), S - 1)
    g16 = pl.multiple_of((idx // 16) * 16, 16)
    xs = _up(R.xn[pl.ds(pl.multiple_of(g16 // 2, 8), 8), :])
    g = _rbf(jnp.dot(xs, _up(R.wgt[...]), preferred_element_type=f32))
    u = _rbf(jnp.dot(xs, _up(R.wut[...]), preferred_element_type=f32))
    g = _rbf(g * jax.nn.sigmoid(g))
    y = _rbf(jnp.dot((g * u).astype(bf16), R.wd[...], preferred_element_type=f32))
    y = _rbf(y * _rbf(jax.nn.sigmoid(rmax[0:1, :])))
    rows = lax.broadcasted_iota(jnp.int32, (16, D), 0)
    R.y[...] = jnp.where(rows == (idx - g16), y, 0.0)
    R.g16[0] = g16


def _run_block(R, blk, prog, pace):
    res = {}
    R.dep = None
    for tok in prog:
        if tok[0] == "a":
            n = int(tok[1])
            _scores(R, blk, *UNITS[n], n % LOOP_SLOTS)
        elif tok[0] == "b":
            n = int(tok[1])
            res[n] = _softmax_pv(R, blk, *UNITS[n], n % LOOP_SLOTS, pace)
            if n % 2 == 1:
                _store_o(R, blk % 2, n // 2, res.pop(n - 1), res.pop(n))
        elif tok == "n":
            _scores(R, blk + 1, *UNITS[0], 0)
        elif tok == "l":
            R.xn_next = _ln_block(R, blk + 1)
        elif tok[0] == "q":
            _proj_k(R, blk + 1, R.xn_next, int(tok[1]))
        elif tok[0] == "v":
            _proj_qv(R, blk + 1, R.xn_next, int(tok[1]))
        elif tok == "O":
            _outproj(R, blk)
        elif tok == "tg":
            _transpose_ffn(R.wg, R.wgt)
        elif tok == "tu":
            _transpose_ffn(R.wu, R.wut)
        elif tok == "f":
            _route_ffn(R)
        else:
            raise ValueError(tok)


def _run_prologue(R, xns, hooks):
    free = list(range(ALL_SLOTS))
    slots, res = {}, {}
    R.dep = None
    for tok in PROG_FIRST:
        if tok in hooks:
            hooks[tok]()
            continue
        if tok == "n":
            free.remove(0)
            _scores(R, 2, *UNITS[0], 0)
            continue
        op, _, bs = tok.partition(".")
        blk = int(bs) if bs else None
        if op[0] == "p":
            _proj_k(R, blk, xns[blk], int(op[1]))
            _proj_qv(R, blk, xns[blk], int(op[1]))
        elif op[0] == "a":
            n = int(op[1])
            slots[blk, n] = max(free)
            free.remove(slots[blk, n])
            _scores(R, blk, *UNITS[n], slots[blk, n])
        elif op[0] == "b":
            n = int(op[1])
            slot = slots.pop((blk, n))
            res[blk, n] = _softmax_pv(R, blk, *UNITS[n], slot, (None, 2)[blk])
            free.append(slot)
            if n % 2 == 1:
                _store_o(R, blk % 2, n // 2, res.pop((blk, n - 1)), res.pop((blk, n)))
        elif op == "O":
            _outproj(R, blk)
        elif op == "l":
            R.xn_next = _ln_block(R, 2)
        elif op[0] == "q":
            _proj_k(R, 2, R.xn_next, int(op[1]))
        elif op[0] == "v":
            _proj_qv(R, 2, R.xn_next, int(op[1]))
        else:
            raise ValueError(tok)


def _kernel(x_hbm, wqkv_hbm, wo_hbm, wr_hbm, wg_hbm, wu_hbm, wd_hbm, o_hbm,
            x, wqkv, wo, wqv, q, k, vt, ot, xn, r, bias, out, wg, wu, wd, wgt, wut, wk, wop,
            s, m, wr, y, g16_ref, sems):
    R = _Ctx()
    R.x, R.wqv, R.wk, R.wo, R.q, R.k, R.vt, R.ot, R.xn, R.r, R.bias = x, wqv, wk, wop, q, k, vt, ot, xn, r, bias
    R.out, R.wg, R.wu, R.wd, R.wgt, R.wut, R.s, R.m, R.y, R.g16 = out, wg, wu, wd, wgt, wut, s, m, y, g16_ref

    def copy(src, dst, i):
        return pltpu.make_async_copy(src, dst, sems.at[i])

    S_X01, S_G0, S_G1, S_G23, S_WO, S_XR, S_FFN, S_OUT, S_LAST, S_PATCH = range(10)

    def wcopy(j, g, sem):
        c0 = j * D + g * 128
        if not isinstance(c0, int):
            c0 = pl.multiple_of(c0, 128)
        return copy(wqkv_hbm.at[:, pl.ds(c0, 128)], wqkv.at[:, pl.ds(c0, 128)], sem)

    x01 = copy(x_hbm.at[0:2 * QB, :], x.at[0:2 * QB, :], S_X01)
    wrcopy = copy(wr_hbm, wr, S_X01)
    wocopy = copy(wo_hbm, wo, S_WO)
    x2copy = copy(x_hbm.at[2 * QB:3 * QB, :], x.at[2 * QB:3 * QB, :], S_WO)
    xrcopy = copy(x_hbm.at[3 * QB:S, :], x.at[3 * QB:S, :], S_XR)
    fcopies = (copy(wg_hbm, wg, S_FFN), copy(wu_hbm, wu, S_FFN), copy(wd_hbm, wd, S_FFN))

    def ocopy(b):
        return copy(out.at[_rows(b), :], o_hbm.at[_rows(b), :], S_OUT)

    x01.start()
    wrcopy.start()

    def start_group(g, carry):
        for j in range(3):
            wcopy(j, g, S_G0 + jnp.minimum(g, 2)).start()
        return carry

    lax.fori_loop(0, 4, start_group, 0)
    wocopy.start()
    x2copy.start()

    jj = lax.broadcasted_iota(jnp.int32, (64, 128), 1) & 63
    rr = lax.broadcasted_iota(jnp.int32, (64, 128), 0)
    bias[0:64, :] = jnp.where(rr > jj, 0.0, NEG)
    bias[64:128, :] = jnp.where(rr <= jj, 0.0, NEG)
    vt[0] = jnp.zeros((D // 2, 128), u32)
    vt[1] = jnp.zeros((D // 2, 128), u32)
    k[0:W // 2, :] = jnp.zeros((W // 2, D), u32)
    x01.wait()
    wrcopy.wait()
    wqv[D:D + 8, :] = _pk(jnp.broadcast_to(wr[...][None, :], (16, D)))
    xns = (_ln_block(R, 0), _ln_block(R, 1))

    def arrive(g):
        for gg in {0: [0], 1: [1], 2: [2, 3], 3: []}[g]:
            for j in range(3):
                wcopy(j, gg, S_G0 + min(gg, 2)).wait()
        if g == 2:
            xrcopy.start()
        gs = slice(g * 128, (g + 1) * 128)
        wqv[g * 64:(g + 1) * 64, :] = _pk(wqkv[:, gs].T)
        wqv[D // 2 + g * 64:D // 2 + (g + 1) * 64, :] = _pk(wqkv[:, 2 * D + g * 128:2 * D + (g + 1) * 128].T)
        wk[:, gs] = _pk(wqkv[:, D + g * 128:D + (g + 1) * 128])

    def wo_arrived():
        wocopy.wait()
        x2copy.wait()
        wop[...] = _pk(wo[...])

    hooks = {f"g{g}": functools.partial(arrive, g) for g in range(4)}
    hooks["w"] = wo_arrived
    _run_prologue(R, xns, hooks)
    ocopy(0).start()
    ocopy(1).start()
    for c in fcopies:
        c.start()

    xrcopy.wait()

    def body(i, carry):
        b = 2 + i
        _run_block(R, b, PROG_LOOP, 1)
        ocopy(b).start()
        return carry

    lax.fori_loop(0, NB - 3, body, 0)

    for c in fcopies:
        c.wait()
    _run_block(R, NB - 1, PROG_LAST, 2)
    g16 = pl.multiple_of(g16_ref[0], 16)
    yv = y[...]
    nw = (NB - 1) * QB
    copy(out.at[0:nw, :], o_hbm.at[0:nw, :], S_OUT).wait()
    cur = out[pl.ds(g16, 16), :].astype(f32)
    out[pl.ds(g16, 16), :] = (cur + yv).astype(bf16)
    last = copy(out.at[nw:S, :], o_hbm.at[nw:S, :], S_LAST)
    last.start()

    @pl.when(g16 < nw)
    def _():
        pc = copy(out.at[pl.ds(g16, 16), :], o_hbm.at[pl.ds(g16, 16), :], S_PATCH)
        pc.start()
        pc.wait()

    last.wait()


@jax.jit
def pallas_parallel_sum__sliding_block__moe_arch_mod__prompt_kernel(
    A_x: jax.Array,
    A_wqkv: jax.Array,
    A_wo: jax.Array,
    B_x: jax.Array,
    B_w_r: jax.Array,
    B_w_gate: jax.Array,
    B_w_up: jax.Array,
    B_w_down: jax.Array,
):
    del B_x
    hbm = lambda a: pltpu.with_memory_space_constraint(a, pltpu.HBM)
    anyspec = pl.BlockSpec(memory_space=pl.ANY)
    out = pl.pallas_call(
        _kernel,
        grid=(),
        in_specs=[anyspec] * 7,
        out_specs=anyspec,
        out_shape=jax.ShapeDtypeStruct((S, D), bf16),
        scratch_shapes=[
            pltpu.VMEM((S, D), bf16),
            pltpu.VMEM((D, 3 * D), bf16),
            pltpu.VMEM((D, D), bf16),
            pltpu.VMEM((D + 8, D), u32),
            pltpu.VMEM((NB, D // 2, 128), u32),
            pltpu.VMEM(((S + W) // 2, D), u32),
            pltpu.VMEM((NB + 2, D // 2, 128), u32),
            pltpu.VMEM((2, D // 2, 128), u32),
            pltpu.VMEM((S // 2, D), u32),
            pltpu.VMEM((NB, 8, 128), f32),
            pltpu.VMEM((128, 128), f32),
            pltpu.VMEM((S, D), bf16),
            pltpu.VMEM((F, D), bf16),
            pltpu.VMEM((F, D), bf16),
            pltpu.VMEM((F, D), bf16),
            pltpu.VMEM((D // 2, F), u32),
            pltpu.VMEM((D // 2, F), u32),
            pltpu.VMEM((D // 2, D), u32),
            pltpu.VMEM((D // 2, D), u32),
            pltpu.VMEM((ALL_SLOTS, 320, 512), f32),
            pltpu.VMEM((ALL_SLOTS, 8, 512), f32),
            pltpu.VMEM((D,), bf16),
            pltpu.VMEM((16, D), f32),
            pltpu.SMEM((1,), jnp.int32),
            pltpu.SemaphoreType.DMA((10,)),
        ],
        compiler_params=pltpu.CompilerParams(
            dimension_semantics=(), vmem_limit_bytes=64 * 1024 * 1024),
        name="sliding_attn_mod_ffn",
    )(hbm(A_x.reshape(S, D)), hbm(A_wqkv), hbm(A_wo), hbm(B_w_r),
      hbm(B_w_gate.T), hbm(B_w_up.T), hbm(B_w_down))
    return out.reshape(1, S, D)
```

```python
import functools

import numpy as np
import jax
import jax.numpy as jnp
from jax import lax
from jax.experimental import pallas as pl
from jax.experimental.pallas import tpu as pltpu

S = 2048
D = 512
H = 32
DH = 16
W = 256
F = 1376
QB = 128
NB = S // QB
NEG = -1e30
QSCALE = (DH ** -0.5) * 1.4426950408889634
EPS_BF16 = float(np.float32(np.asarray(1e-5, dtype=jnp.bfloat16)))
f32 = jnp.float32
bf16 = jnp.bfloat16
u32 = jnp.uint32
NT = (((1,), (1,)), ((), ()))
TN = (((0,), (0,)), ((), ()))

UNITS = [(g, half) for g in range(4) for half in range(2)]

PROG_FIRST = ("g0 p0.1 p0.0 g1 a0.1 p1.0 a0.0 p1.1 a1.0 b0.0 a1.1 b1.0 b0.1 a2.0 a2.1 b1.1 a3.1 b2.0 "
              "g2 a3.0 p2.0 g3 p2.1 b2.1 p3.1 a4.0 a5.0 p3.0 b3.1 b3.0 a4.1 a5.1 b4.0 b5.0 a6.0 a7.0 b4.1 "
              "w b5.1 l b6.0 a6.1 a7.1 q0 q1 v0 b7.0 q2 v3 b6.1 n v1 q3 b7.1 O.0 O.1 v2").split()
PROG_LOOP = "a1 b0 a2 b1 a3 b2 a4 b3 a5 b4 a6 b5 a7 l q0 b6 q1 v3 v0 v2 b7 q2 v1 n O q3".split()
PROG_LAST = "tg tu a1 b0 a2 b1 a3 b2 a4 b3 a5 b4 a6 b5 a7 b6 b7 f O".split()
LOOP_SLOTS = 3
ALL_SLOTS = 4


def _rbf(x):
    return x.astype(bf16).astype(f32)


def _pk(x):
    return pltpu.bitcast(x, u32)


def _up(x):
    return pltpu.bitcast(x, bf16)


def _prow(start, n):
    if isinstance(start, int):
        return pl.ds(start // 2, n // 2)
    return pl.ds(pl.multiple_of(start // 2, 8), n // 2)


def _rows(blk):
    if isinstance(blk, int):
        return pl.ds(blk * QB, QB)
    return pl.ds(pl.multiple_of(blk * QB, QB), QB)


def _layernorm(x):
    xf = x.astype(f32)
    mean = jnp.mean(xf, axis=-1, keepdims=True)
    c = xf - mean
    var = jnp.mean(c * c, axis=-1, keepdims=True)
    den = _rbf(jnp.sqrt(_rbf(_rbf(var) + EPS_BF16)))
    xc = _rbf(xf - _rbf(mean))
    return (xc * (1.0 / den)).astype(bf16)


class _Ctx:
    pass


def _ln_block(R, blk):
    xn = _layernorm(R.x[_rows(blk), :])
    R.xn[_prow(blk * QB, QB), :] = _pk(xn)
    return xn


def _proj_k(R, blk, xn, g):
    c0, c1 = g * 128, (g + 1) * 128
    kk = jnp.dot(xn, _up(R.wk[:, c0:c1]), preferred_element_type=f32)
    R.k[_prow((blk + 2) * QB, QB), c0:c1] = _pk(kk.astype(bf16))


def _proj_qv(R, blk, xn, g):
    lhs = [_up(R.wqv[g * 64:(g + 1) * 64, :]), _up(R.wqv[D // 2 + g * 64:D // 2 + (g + 1) * 64, :])]
    if g == 3:
        lhs.append(_up(R.wqv[D:D + 8, :]))
    qv = lax.dot_general(jnp.concatenate(lhs, axis=0), xn, NT, preferred_element_type=f32)
    qt = _pk((qv[0:128] * QSCALE).astype(bf16))
    parts = [qt[8 * h:8 * h + 8] if h % 2 == 0 else pltpu.roll(qt[8 * h:8 * h + 8], 64, 1) for h in range(8)]
    R.q[blk, 64 * g:64 * (g + 1), :] = jnp.concatenate(parts, axis=0)
    R.vt[blk + 2, g * 64:(g + 1) * 64, :] = _pk(qv[128:256].astype(bf16))
    if g == 3:
        R.r[blk] = qv[256:264]


def _scores(R, blk, g, half, slot):
    w0 = 64 * half
    lo = lax.broadcasted_iota(jnp.int32, (8, 128), 1) < 64
    mlo = jnp.where(lo, np.uint32(0xFFFFFFFF), np.uint32(0))
    mhi = jnp.where(lo, np.uint32(0), np.uint32(0xFFFFFFFF))
    ma, mb = (mlo, mhi) if half == 0 else (mhi, mlo)
    qcols = []
    for p in range(4):
        h0 = 8 * g + 2 * p
        a = R.q[blk, 8 * h0:8 * h0 + 8, :] & ma
        b = R.q[blk, 8 * h0 + 8:8 * h0 + 16, :] & mb
        rows = []
        if p > 0:
            rows.append(jnp.zeros((16 * p, 128), u32))
        rows += [a, b]
        if p < 3:
            rows.append(jnp.zeros((48 - 16 * p, 128), u32))
        qcols.append(jnp.concatenate(rows, axis=0))
    qbd = _up(jnp.concatenate(qcols, axis=1))
    c_lo = max(0, (W - QB * blk - w0) // 64) if isinstance(blk, int) else 0
    kblk = _up(R.k[_prow(blk * QB + w0 + 64 * c_lo, 320 - 64 * c_lo), g * 128:(g + 1) * 128])
    st = jnp.dot(kblk, qbd, preferred_element_type=f32)
    cols, ms = [], []
    for p in range(4):
        pieces, pm = [], None
        for c in range(5):
            if c < c_lo:
                pieces.append(None)
                continue
            sc = st[(c - c_lo) * 64:(c - c_lo + 1) * 64, p * 128:(p + 1) * 128]
            if c == 0:
                sc = sc + R.bias[0:64, :]
            elif c == 4:
                sc = sc + R.bias[64:128, :]
            pieces.append(sc)
            cm = jnp.max(sc.reshape(8, 8, 128), axis=0)
            pm = cm if pm is None else jnp.maximum(pm, cm)
        cols.append(pieces)
        ms.append(jnp.max(pm, axis=0, keepdims=True))
    R.dep = [[None if cols[p][c] is None else cols[p][c][0:8, :] for c in range(5)] for p in range(4)]
    for p in range(4):
        for c in range(5):
            if cols[p][c] is not None:
                R.s[slot, c * 64:(c + 1) * 64, p * 128:(p + 1) * 128] = cols[p][c]
        R.m[slot, :, p * 128:(p + 1) * 128] = jnp.broadcast_to(ms[p], (8, 128))


def _softmax_pv(R, blk, g, half, slot, pace):
    dep, R.dep = R.dep, None
    w0 = 64 * half
    first_valid = W - QB * blk if isinstance(blk, int) else 0
    cols = [[R.s[slot, c * 64:(c + 1) * 64, p * 128:(p + 1) * 128] if w0 + 64 * c >= first_valid else None
             for c in range(5)] for p in range(4)]
    ms = [R.m[slot, 0:1, p * 128:(p + 1) * 128] for p in range(4)]
    accs, ls = [None] * 4, [None] * 4
    z = jnp.zeros((64, 128), f32)
    for t in range(3):
        for p in range(4):
            es = []
            for c2 in range(2):
                wrow = 128 * t + 64 * c2
                c = (wrow - w0) // 64
                if c < 0 or c > 4 or wrow < first_valid:
                    es.append(z)
                    continue
                cd = c - (pace or 0)
                if pace is not None and dep is not None and 0 <= cd < 5 and dep[p][cd] is not None:
                    mc = (ms[p] + 0.0 * dep[p][cd])[None]
                    e = jnp.exp2(cols[p][c].reshape(8, 8, 128) - mc).reshape(64, 128)
                else:
                    e = jnp.exp2(cols[p][c] - ms[p])
                es.append(e)
                part = jnp.sum(e.reshape(8, 8, 128), axis=0)
                ls[p] = part if ls[p] is None else ls[p] + part
            if 128 * (t + 1) <= first_valid:
                continue
            hp = g * 8 + 2 * p
            pt = jnp.concatenate(es, axis=0).astype(bf16)
            vt = _up(R.vt[blk + t, hp * (DH // 2):(hp + 2) * (DH // 2), :])
            o = jnp.dot(vt, pt, preferred_element_type=f32)
            accs[p] = o if accs[p] is None else accs[p] + o
    return [accs[p] * (1.0 / jnp.sum(ls[p], axis=0, keepdims=True)) for p in range(4)]


def _store_o(R, slot, g, oas, obs):
    lo = lax.broadcasted_iota(jnp.int32, (DH, 128), 1) < 64
    for p in range(4):
        hp = g * 8 + 2 * p
        oa, ob = oas[p], obs[p]
        o0 = jnp.where(lo, oa[:DH], ob[:DH])
        o1 = pltpu.roll(jnp.where(lo, ob[DH:], oa[DH:]), 64, 1)
        R.ot[slot, hp * (DH // 2):(hp + 2) * (DH // 2), :] = _pk(jnp.concatenate([o0, o1], axis=0).astype(bf16))


def _outproj(R, blk):
    ao = lax.dot_general(_up(R.ot[blk % 2]), _up(R.wo[...]), TN, preferred_element_type=f32)
    x = R.x[_rows(blk), :].astype(f32)
    xn = _up(R.xn[_prow(blk * QB, QB), :]).astype(f32)
    R.out[_rows(blk), :] = (x + ao + xn).astype(bf16)


def _transpose_ffn(src, dst):
    for j in range(pl.cdiv(F, 128)):
        n = min(128, F - 128 * j)
        dst[:, 128 * j:128 * j + n] = _pk(src[128 * j:128 * j + n, :].T)


def _route_ffn(R):
    r = _rbf(R.r[...])
    pos = (lax.broadcasted_iota(jnp.int32, r.shape, 0) * QB + lax.broadcasted_iota(jnp.int32, r.shape, 2))
    rmax = jnp.max(jnp.max(r, axis=0), axis=1, keepdims=True)
    idx = jnp.minimum(jnp.min(jnp.where(r == rmax[None], pos, S)), S - 1)
    g16 = pl.multiple_of((idx // 16) * 16, 16)
    xs = _up(R.xn[pl.ds(pl.multiple_of(g16 // 2, 8), 8), :])
    g = _rbf(jnp.dot(xs, _up(R.wgt[...]), preferred_element_type=f32))
    u = _rbf(jnp.dot(xs, _up(R.wut[...]), preferred_element_type=f32))
    g = _rbf(g * jax.nn.sigmoid(g))
    y = _rbf(jnp.dot((g * u).astype(bf16), R.wd[...], preferred_element_type=f32))
    y = _rbf(y * _rbf(jax.nn.sigmoid(rmax[0:1, :])))
    rows = lax.broadcasted_iota(jnp.int32, (16, D), 0)
    R.y[...] = jnp.where(rows == (idx - g16), y, 0.0)
    R.g16[0] = g16


def _run_block(R, blk, prog, pace):
    res = {}
    R.dep = None
    for tok in prog:
        if tok[0] == "a":
            n = int(tok[1])
            _scores(R, blk, *UNITS[n], n % LOOP_SLOTS)
        elif tok[0] == "b":
            n = int(tok[1])
            res[n] = _softmax_pv(R, blk, *UNITS[n], n % LOOP_SLOTS, pace)
            if n % 2 == 1:
                _store_o(R, blk % 2, n // 2, res.pop(n - 1), res.pop(n))
        elif tok == "n":
            _scores(R, blk + 1, *UNITS[0], 0)
        elif tok == "l":
            R.xn_next = _ln_block(R, blk + 1)
        elif tok[0] == "q":
            _proj_k(R, blk + 1, R.xn_next, int(tok[1]))
        elif tok[0] == "v":
            _proj_qv(R, blk + 1, R.xn_next, int(tok[1]))
        elif tok == "O":
            _outproj(R, blk)
        elif tok == "tg":
            _transpose_ffn(R.wg, R.wgt)
        elif tok == "tu":
            _transpose_ffn(R.wu, R.wut)
        elif tok == "f":
            _route_ffn(R)
        else:
            raise ValueError(tok)


def _run_prologue(R, xns, hooks):
    free = list(range(ALL_SLOTS))
    slots, res = {}, {}
    R.dep = None
    for tok in PROG_FIRST:
        if tok in hooks:
            hooks[tok]()
            continue
        if tok == "n":
            free.remove(0)
            _scores(R, 2, *UNITS[0], 0)
            continue
        op, _, bs = tok.partition(".")
        blk = int(bs) if bs else None
        if op[0] == "p":
            _proj_k(R, blk, xns[blk], int(op[1]))
            _proj_qv(R, blk, xns[blk], int(op[1]))
        elif op[0] == "a":
            n = int(op[1])
            slots[blk, n] = max(free)
            free.remove(slots[blk, n])
            _scores(R, blk, *UNITS[n], slots[blk, n])
        elif op[0] == "b":
            n = int(op[1])
            slot = slots.pop((blk, n))
            res[blk, n] = _softmax_pv(R, blk, *UNITS[n], slot, (None, 2)[blk])
            free.append(slot)
            if n % 2 == 1:
                _store_o(R, blk % 2, n // 2, res.pop((blk, n - 1)), res.pop((blk, n)))
        elif op == "O":
            _outproj(R, blk)
        elif op == "l":
            R.xn_next = _ln_block(R, 2)
        elif op[0] == "q":
            _proj_k(R, 2, R.xn_next, int(op[1]))
        elif op[0] == "v":
            _proj_qv(R, 2, R.xn_next, int(op[1]))
        else:
            raise ValueError(tok)


def _kernel(x_hbm, wqkv_hbm, wo_hbm, wr_hbm, wg_hbm, wu_hbm, wd_hbm, o_hbm,
            x, wqkv, wo, wqv, q, k, vt, ot, xn, r, bias, out, wg, wu, wd, wgt, wut, wk, wop,
            s, m, wr, y, g16_ref, sems):
    R = _Ctx()
    R.x, R.wqv, R.wk, R.wo, R.q, R.k, R.vt, R.ot, R.xn, R.r, R.bias = x, wqv, wk, wop, q, k, vt, ot, xn, r, bias
    R.out, R.wg, R.wu, R.wd, R.wgt, R.wut, R.s, R.m, R.y, R.g16 = out, wg, wu, wd, wgt, wut, s, m, y, g16_ref

    def copy(src, dst, i):
        return pltpu.make_async_copy(src, dst, sems.at[i])

    S_X01, S_G0, S_G1, S_G23, S_WO, S_XR, S_FFN, S_OUT, S_LAST, S_PATCH = range(10)

    def wcopy(j, g, sem):
        c0 = j * D + g * 128
        if not isinstance(c0, int):
            c0 = pl.multiple_of(c0, 128)
        return copy(wqkv_hbm.at[:, pl.ds(c0, 128)], wqkv.at[:, pl.ds(c0, 128)], sem)

    x01 = copy(x_hbm.at[0:2 * QB, :], x.at[0:2 * QB, :], S_X01)
    wrcopy = copy(wr_hbm, wr, S_X01)
    wocopy = copy(wo_hbm, wo, S_WO)
    x2copy = copy(x_hbm.at[2 * QB:3 * QB, :], x.at[2 * QB:3 * QB, :], S_WO)
    xrcopy = copy(x_hbm.at[3 * QB:S, :], x.at[3 * QB:S, :], S_XR)
    fcopies = (copy(wg_hbm, wg, S_FFN), copy(wu_hbm, wu, S_FFN), copy(wd_hbm, wd, S_FFN))

    def ocopy(b):
        return copy(out.at[_rows(b), :], o_hbm.at[_rows(b), :], S_OUT)

    x01.start()
    wrcopy.start()

    def start_group(g, carry):
        for j in range(3):
            wcopy(j, g, S_G0 + jnp.minimum(g, 2)).start()
        return carry

    lax.fori_loop(0, 4, start_group, 0)
    wocopy.start()
    x2copy.start()

    jj = lax.broadcasted_iota(jnp.int32, (64, 128), 1) & 63
    rr = lax.broadcasted_iota(jnp.int32, (64, 128), 0)
    bias[0:64, :] = jnp.where(rr > jj, 0.0, NEG)
    bias[64:128, :] = jnp.where(rr <= jj, 0.0, NEG)
    vt[0] = jnp.zeros((D // 2, 128), u32)
    vt[1] = jnp.zeros((D // 2, 128), u32)
    k[0:W // 2, :] = jnp.zeros((W // 2, D), u32)
    x01.wait()
    wrcopy.wait()
    wqv[D:D + 8, :] = _pk(jnp.broadcast_to(wr[...][None, :], (16, D)))
    xns = (_ln_block(R, 0), _ln_block(R, 1))

    def arrive(g):
        for gg in {0: [0], 1: [1], 2: [2, 3], 3: []}[g]:
            for j in range(3):
                wcopy(j, gg, S_G0 + min(gg, 2)).wait()
        if g == 2:
            xrcopy.start()
        gs = slice(g * 128, (g + 1) * 128)
        wqv[g * 64:(g + 1) * 64, :] = _pk(wqkv[:, gs].T)
        wqv[D // 2 + g * 64:D // 2 + (g + 1) * 64, :] = _pk(wqkv[:, 2 * D + g * 128:2 * D + (g + 1) * 128].T)
        wk[:, gs] = _pk(wqkv[:, D + g * 128:D + (g + 1) * 128])

    def wo_arrived():
        wocopy.wait()
        x2copy.wait()
        wop[...] = _pk(wo[...])

    hooks = {f"g{g}": functools.partial(arrive, g) for g in range(4)}
    hooks["w"] = wo_arrived
    _run_prologue(R, xns, hooks)
    ocopy(0).start()
    ocopy(1).start()
    for c in fcopies:
        c.start()

    xrcopy.wait()

    def body(i, carry):
        b = 2 + i
        _run_block(R, b, PROG_LOOP, 1)
        ocopy(b).start()
        return carry

    lax.fori_loop(0, NB - 3, body, 0)

    for c in fcopies:
        c.wait()
    _run_block(R, NB - 1, PROG_LAST, 2)
    g16 = pl.multiple_of(g16_ref[0], 16)
    yv = y[...]
    nw = (NB - 1) * QB
    copy(out.at[0:nw, :], o_hbm.at[0:nw, :], S_OUT).wait()
    cur = out[pl.ds(g16, 16), :].astype(f32)
    out[pl.ds(g16, 16), :] = (cur + yv).astype(bf16)
    last = copy(out.at[nw:S, :], o_hbm.at[nw:S, :], S_LAST)
    last.start()

    @pl.when(g16 < nw)
    def _():
        pc = copy(out.at[pl.ds(g16, 16), :], o_hbm.at[pl.ds(g16, 16), :], S_PATCH)
        pc.start()
        pc.wait()

    last.wait()


@jax.jit
def pallas_parallel_sum__sliding_block__moe_arch_mod__prompt_kernel(
    A_x: jax.Array,
    A_wqkv: jax.Array,
    A_wo: jax.Array,
    B_x: jax.Array,
    B_w_r: jax.Array,
    B_w_gate: jax.Array,
    B_w_up: jax.Array,
    B_w_down: jax.Array,
):
    del B_x
    hbm = lambda a: pltpu.with_memory_space_constraint(a, pltpu.HBM)
    anyspec = pl.BlockSpec(memory_space=pl.ANY)
    out = pl.pallas_call(
        _kernel,
        grid=(),
        in_specs=[anyspec] * 7,
        out_specs=anyspec,
        out_shape=jax.ShapeDtypeStruct((S, D), bf16),
        scratch_shapes=[
            pltpu.VMEM((S, D), bf16),
            pltpu.VMEM((D, 3 * D), bf16),
            pltpu.VMEM((D, D), bf16),
            pltpu.VMEM((D + 8, D), u32),
            pltpu.VMEM((NB, D // 2, 128), u32),
            pltpu.VMEM(((S + W) // 2, D), u32),
            pltpu.VMEM((NB + 2, D // 2, 128), u32),
            pltpu.VMEM((2, D // 2, 128), u32),
            pltpu.VMEM((S // 2, D), u32),
            pltpu.VMEM((NB, 8, 128), f32),
            pltpu.VMEM((128, 128), f32),
            pltpu.VMEM((S, D), bf16),
            pltpu.VMEM((F, D), bf16),
            pltpu.VMEM((F, D), bf16),
            pltpu.VMEM((F, D), bf16),
            pltpu.VMEM((D // 2, F), u32),
            pltpu.VMEM((D // 2, F), u32),
            pltpu.VMEM((D // 2, D), u32),
            pltpu.VMEM((D // 2, D), u32),
            pltpu.VMEM((ALL_SLOTS, 320, 512), f32),
            pltpu.VMEM((ALL_SLOTS, 8, 512), f32),
            pltpu.VMEM((D,), bf16),
            pltpu.VMEM((16, D), f32),
            pltpu.SMEM((1,), jnp.int32),
            pltpu.SemaphoreType.DMA((10,)),
        ],
        compiler_params=pltpu.CompilerParams(
            dimension_semantics=(), vmem_limit_bytes=64 * 1024 * 1024),
        name="sliding_attn_mod_ffn",
    )(hbm(A_x.reshape(S, D)), hbm(A_wqkv), hbm(A_wo), hbm(B_w_r),
      hbm(B_w_gate.T), hbm(B_w_up.T), hbm(B_w_down))
    return out.reshape(1, S, D)
```
